```python
import os as _os
_os.environ.setdefault("JAX_PLATFORMS", "cpu")
import jax
import jax.numpy as jnp

def _softmax(x, axis=-1):
    return jax.nn.softmax(x, axis=axis)
def _gelu(x):
    return jax.nn.gelu(x, approximate=True)
def _silu(x):
    return jax.nn.silu(x)
def _sigmoid(x):
    return jax.nn.sigmoid(x)
def _layernorm(x, axis=-1, eps=1e-5):
    m = jnp.mean(x, axis=axis, keepdims=True)
    v = jnp.var(x, axis=axis, keepdims=True)
    return (x - m) / jnp.sqrt(v + eps)
def _scatter_add(tgt, idx, src, axis=0):
    return tgt.at[idx].add(src)
def _segment_sum(src, seg, n):
    return jax.ops.segment_sum(src, seg, n)
class _Rng:
    def __init__(self, key):
        self._k = key
    def _next(self):
        self._k, sub = jax.random.split(self._k)
        return sub
    def normal(self, shape):
        return jax.random.normal(self._next(), shape, dtype=jnp.bfloat16)
    def randint(self, lo, hi, shape):
        return jax.random.randint(self._next(), shape, lo, hi, dtype=jnp.int32)
    def uniform(self, shape, lo=0.0, hi=1.0):
        return jax.random.uniform(self._next(), shape, jnp.bfloat16, lo, hi)
    def permutation(self, n):
        return jax.random.permutation(self._next(), n)


kernel_name = 'gated_mix__linear_attn_block__glu_gated_swiglu__prompt'

def setup_inputs():
    _rng = _Rng(jax.random.key(int.from_bytes(__import__("os").urandom(4), "little")))
    _w = (lambda a: (lambda t: t.astype(jnp.bfloat16) if jnp.issubdtype(t.dtype, jnp.floating) else t)(jnp.asarray(a)))
    def _A_setup():
        B, S, D = 1, 2048, 1024
        return {
            "x": _w((lambda *s: _rng.normal(s) * 0.05)(B, S, D)),
            "wqkv": _w((lambda *s: _rng.normal(s) * 0.8)(D, 3 * D)),
            "wo": _w((lambda *s: _rng.normal(s) * 0.05)(D, D)),
        }
    _A_in = _A_setup()

    def _B_setup():
        B, S, D, F = 1, 2048, 1024, 3584
        return {
            "x": _w((lambda *s: _rng.normal(s) * 0.05)(B, S, D)),
            "w1": _w((lambda *s: _rng.normal(s) * 1.6)(D, F) * (2.0 / D) ** 0.5),
            "w3": _w((lambda *s: _rng.normal(s) * 1.6)(D, F) * (2.0 / D) ** 0.5),
            "w2": _w((lambda *s: _rng.normal(s) * 1.6)(F, D) * (2.0 / F) ** 0.5),
        }
    _B_in = _B_setup()

    return {
        "A_x": _A_in["x"],
        "A_wqkv": _A_in["wqkv"],
        "A_wo": _A_in["wo"],
        "B_x": _B_in["x"],
        "B_w1": _B_in["w1"],
        "B_w3": _B_in["w3"],
        "B_w2": _B_in["w2"],
        "gate_w": _w((lambda *s: _rng.normal(s) * 0.05)(1024) * 16.0),
    }

def reference(A_x, A_wqkv, A_wo, B_x, B_w1, B_w3, B_w2, gate_w):
    def _A_ref(x, wqkv, wo):
        B, S, D = x.shape
        H = 32; Dh = D // H
        qkv = (lambda x, *d: x.transpose(*d))((x @ wqkv).reshape(B, S, 3, H, Dh), 2, 0, 3, 1, 4)
        q, k, v = qkv[0], qkv[1], qkv[2]
        phi = lambda t: jnp.where(t > 0, t + 1, jnp.exp(t)) + 1e-6
        pq, pk = phi(q), phi(k)
        kv = jnp.einsum("bhsd,bhse->bhde", pk, v)
        z = jnp.einsum("bhsd->bhd", pk)
        num = jnp.einsum("bhqd,bhde->bhqe", pq, kv)
        den = jnp.einsum("bhqd,bhd->bhq", pq, z)[..., None] + 1e-6
        o = num / den
        return (lambda x, *d: x.transpose(*d))(o, 0, 2, 1, 3).reshape(B, S, D) @ wo

    def _B_ref(x, w1, w3, w2):
        gate = jnp.einsum("bsd,df->bsf", x, w1)
        up = jnp.einsum("bsd,df->bsf", x, w3)
        h = _silu(gate) * up
        out = jnp.einsum("bsf,fd->bsd", h, w2)
        return out

    x = A_x
    g = _sigmoid((x * gate_w).sum(-1, keepdims=True))
    a = _A_ref(x, A_wqkv, A_wo)
    b = _B_ref(x, B_w1, B_w3, B_w2)
    return g * a + (1 - g) * b
```

```python
import jax
import jax.numpy as jnp
from jax import lax
import jax.experimental.pallas as pl
import jax.experimental.pallas.tpu as pltpu

_H = 32
_LANE = 128


def _phi(t):
    return jnp.where(t > 0, t + 1.0, jnp.exp(t)) + 1e-6


def _make_kernel(S, D, F, TM, NF, widths, ahead):
    NT = S // TM
    NB = D // _LANE
    DH = D // _H
    TF = F // NF
    TA = D // NF
    NC = len(widths)
    starts = [sum(widths[:c]) for c in range(NC)]
    assert sum(widths) == D and NT >= 2 and NC >= 2
    assert TA % _LANE == 0 and TF % _LANE == 0 and _LANE % DH == 0
    f32, bf16 = jnp.float32, jnp.bfloat16

    def kernel(gw_ref, x_hbm, wqkv_hbm, wo_hbm, w1_hbm, w3_hbm, w2_hbm, o_ref,
               x_v, pq_v, g_v, wq_v, wk_v, wv_v, wo_v, w1_v, w3_v, w2_v,
               kv_acc, z_acc, m_v, zb_v, acc, xsem, csem, wsem, fsem):
        p = pl.program_id(0)
        i = pl.program_id(1)

        def cp_x(t):
            return pltpu.make_async_copy(x_hbm.at[pl.ds(t * TM, TM), :],
                                         x_v.at[pl.ds(t * TM, TM), :], xsem.at[t])

        def cp_chunk(c):
            return [pltpu.make_async_copy(
                        wqkv_hbm.at[:, pl.ds((m + 1) * D + starts[c], widths[c])],
                        dst.at[:, pl.ds(starts[c], widths[c])],
                        csem.at[2 * c + m])
                    for m, dst in enumerate((wk_v, wv_v))]

        cp_wo = pltpu.make_async_copy(wo_hbm, wo_v, wsem.at[0])
        cp_wq = pltpu.make_async_copy(wqkv_hbm.at[:, pl.ds(0, D)], wq_v, wsem.at[1])

        def cp_ffn(c):
            return (
                pltpu.make_async_copy(w1_hbm.at[:, pl.ds(c * TF, TF)], w1_v.at[c], fsem.at[3 * c]),
                pltpu.make_async_copy(w3_hbm.at[:, pl.ds(c * TF, TF)], w3_v.at[c], fsem.at[3 * c + 1]),
                pltpu.make_async_copy(w2_hbm.at[pl.ds(c * TF, TF), :], w2_v.at[c], fsem.at[3 * c + 2]),
            )

        def gate(x, row0):
            gl = jnp.sum(x.astype(f32) * gw_ref[...].astype(f32), axis=1, keepdims=True)
            g_v[pl.ds(row0, TM), :] = jax.nn.sigmoid(gl)

        def q_cols(x, tix):
            q = jnp.dot(x, wq_v[...], preferred_element_type=f32)
            pqT = _phi(q).T.astype(bf16)
            for c in range(NF):
                pq_v[tix * NF + c] = pqT[c * TA:(c + 1) * TA, :]

        def kv_cols(x, c0, w, first):
            k = jnp.dot(x, wk_v[:, c0:c0 + w], preferred_element_type=f32)
            pkT = _phi(k).T
            zs = pkT[:, 0:_LANE]
            for c in range(1, TM // _LANE):
                zs = zs + pkT[:, c * _LANE:(c + 1) * _LANE]
            if first:
                z_acc[c0:c0 + w, :] = zs
            else:
                z_acc[c0:c0 + w, :] += zs
            pkT = pkT.astype(bf16)
            v = jnp.dot(x, wv_v[:, c0:c0 + w], preferred_element_type=f32).astype(bf16)
            for j in range(w // _LANE):
                sl = slice(j * _LANE, (j + 1) * _LANE)
                gsl = slice(c0 + j * _LANE, c0 + (j + 1) * _LANE)
                t = jnp.dot(pkT[sl, :], v[:, sl], preferred_element_type=f32)
                if first:
                    kv_acc[gsl, :] = t
                else:
                    kv_acc[gsl, :] += t

        @pl.when(jnp.logical_and(p == 0, i == 0))
        def _():
            cp_x(0).start()
            for c in range(min(ahead, NC)):
                for cp in cp_chunk(c):
                    cp.start()
            cp_x(0).wait()
            x = x_v[pl.ds(0, TM), :]
            gate(x, 0)
            for c in range(NC):
                for cp in cp_chunk(c):
                    cp.wait()
                if c + ahead < NC:
                    for cp in cp_chunk(c + ahead):
                        cp.start()
                if c == NC - 2:
                    cp_wq.start()
                if c == NC - 1:
                    cp_x(1).start()
                kv_cols(x, starts[c], widths[c], True)
            cp_wq.wait()
            for t in range(2, NT):
                cp_x(t).start()
            q_cols(x, 0)

        @pl.when(jnp.logical_and(p == 0, i > 0))
        def _():
            cp_x(i).wait()

            @pl.when(i == 1)
            def _():
                cp_wo.start()
                for c in range(NF):
                    for cp in cp_ffn(c):
                        cp.start()

            row0 = pl.multiple_of(i * TM, TM)
            x = x_v[pl.ds(row0, TM), :]
            gate(x, row0)
            q_cols(x, i)
            kv_cols(x, 0, D, False)

        @pl.when(jnp.logical_and(p == 1, i == 0))
        def _():
            cp_wo.wait()
            r = lax.broadcasted_iota(jnp.int32, (_LANE, _LANE), 0) // DH
            c = lax.broadcasted_iota(jnp.int32, (_LANE, _LANE), 1) // DH
            same_head = r == c
            for j in range(NB):
                sl = slice(j * _LANE, (j + 1) * _LANE)
                cc, off = divmod(j * _LANE, TA)
                lsl = slice(off, off + _LANE)
                kvb = jnp.where(same_head, kv_acc[sl, :], 0.0).astype(bf16)
                m_v[cc, lsl, :] = jnp.dot(kvb, wo_v[sl, :], preferred_element_type=f32).astype(bf16)
                z = jnp.sum(z_acc[sl, :], axis=1, keepdims=True)
                zb_v[cc, lsl, :] = jnp.broadcast_to(z.astype(bf16).astype(f32), (_LANE, _LANE))
            for c in range(NF):
                for cp in cp_ffn(c):
                    cp.wait()

        @pl.when(p == 1)
        def _():
            row0 = pl.multiple_of(i * TM, TM)
            acc[...] = jnp.zeros_like(acc)

            def body(c, carry):
                x = x_v[pl.ds(row0, TM), :]
                g = g_v[pl.ds(row0, TM), :]
                pqT = pq_v[i * NF + c].astype(f32)
                zb = zb_v[c]
                zz = jnp.concatenate([zb] * (TM // _LANE), axis=1)
                prod = (pqT * zz).reshape(TA // DH, DH, TM)
                den = jnp.sum(prod, axis=1, keepdims=True) + 1e-6
                pnT = (pqT.reshape(TA // DH, DH, TM) / den).reshape(TA, TM)
                pn = (pnT.T * g).astype(bf16)
                gt = jnp.dot(x, w1_v[c], preferred_element_type=f32)
                up = jnp.dot(x, w3_v[c], preferred_element_type=f32)
                h = (gt * jax.nn.sigmoid(gt) * up * (1.0 - g)).astype(bf16)
                acc[...] += (jnp.dot(pn, m_v[c], preferred_element_type=f32)
                             + jnp.dot(h, w2_v[c], preferred_element_type=f32))
                return carry

            lax.fori_loop(0, NF, body, 0)
            o_ref[...] = acc[...].astype(o_ref.dtype)

    return kernel, NT, NC, TF, TA


@jax.jit
def pallas_gated_mix__linear_attn_block__glu_gated_swiglu__prompt_kernel(
    A_x: jax.Array,
    A_wqkv: jax.Array,
    A_wo: jax.Array,
    B_x: jax.Array,
    B_w1: jax.Array,
    B_w3: jax.Array,
    B_w2: jax.Array,
    gate_w: jax.Array,
):
    B, S, D = A_x.shape
    assert B == 1
    F = B_w1.shape[1]
    TM, NF = 256, 2
    widths = [128, 128, 256, 256, 256]
    kernel, NT, NC, TF, TA = _make_kernel(S, D, F, TM, NF, widths, 2)
    bf16, f32 = jnp.bfloat16, jnp.float32

    x2 = A_x.reshape(S, D)
    gw = gate_w.reshape(1, D)
    any_spec = pl.BlockSpec(memory_space=pl.ANY)
    out = pl.pallas_call(
        kernel,
        grid=(2, NT),
        in_specs=[
            pl.BlockSpec((1, D), lambda p, i: (0, 0)),
            any_spec, any_spec, any_spec, any_spec, any_spec, any_spec,
        ],
        out_specs=pl.BlockSpec((TM, D), lambda p, i: (i * p, 0)),
        out_shape=jax.ShapeDtypeStruct((S, D), A_x.dtype),
        scratch_shapes=[
            pltpu.VMEM((S, D), bf16),
            pltpu.VMEM((NT * NF, TA, TM), bf16),
            pltpu.VMEM((S, 1), f32),
            pltpu.VMEM((D, D), bf16),
            pltpu.VMEM((D, D), bf16),
            pltpu.VMEM((D, D), bf16),
            pltpu.VMEM((D, D), bf16),
            pltpu.VMEM((NF, D, TF), bf16),
            pltpu.VMEM((NF, D, TF), bf16),
            pltpu.VMEM((NF, TF, D), bf16),
            pltpu.VMEM((D, _LANE), f32),
            pltpu.VMEM((D, _LANE), f32),
            pltpu.VMEM((NF, TA, D), bf16),
            pltpu.VMEM((NF, TA, _LANE), f32),
            pltpu.VMEM((TM, D), f32),
            pltpu.SemaphoreType.DMA((NT,)),
            pltpu.SemaphoreType.DMA((2 * NC,)),
            pltpu.SemaphoreType.DMA((2,)),
            pltpu.SemaphoreType.DMA((3 * NF,)),
        ],
        compiler_params=pltpu.CompilerParams(
            dimension_semantics=("arbitrary", "arbitrary"),
            vmem_limit_bytes=100 * 1024 * 1024,
        ),
    )(gw, x2, A_wqkv, A_wo, B_w1, B_w3, B_w2)
    return out.reshape(B, S, D)
```

```python
import jax
import jax.numpy as jnp
from jax import lax
import jax.experimental.pallas as pl
import jax.experimental.pallas.tpu as pltpu

_H = 32
_LANE = 128


def _phi(t):
    return jnp.where(t > 0, t + 1.0, jnp.exp(t)) + 1e-6


def _make_kernel(S, D, F, TM, NF, widths, ahead):
    NT = S // TM
    NB = D // _LANE
    DH = D // _H
    TF = F // NF
    TA = D // NF
    NC = len(widths)
    starts = [sum(widths[:c]) for c in range(NC)]
    assert sum(widths) == D and NT >= 2 and NC >= 2
    assert TA % _LANE == 0 and TF % _LANE == 0 and _LANE % DH == 0
    f32, bf16 = jnp.float32, jnp.bfloat16

    def kernel(gw_ref, x_hbm, wqkv_hbm, wo_hbm, w1_hbm, w3_hbm, w2_hbm, o_ref,
               x_v, pq_v, g_v, wq_v, wk_v, wv_v, wo_v, w1_v, w3_v, w2_v,
               kv_acc, z_acc, m_v, zb_v, acc, xsem, csem, wsem, fsem):
        p = pl.program_id(0)
        i = pl.program_id(1)

        def cp_x(t):
            return pltpu.make_async_copy(x_hbm.at[pl.ds(t * TM, TM), :],
                                         x_v.at[pl.ds(t * TM, TM), :], xsem.at[t])

        def cp_chunk(c):
            return [pltpu.make_async_copy(
                        wqkv_hbm.at[:, pl.ds((m + 1) * D + starts[c], widths[c])],
                        dst.at[:, pl.ds(starts[c], widths[c])],
                        csem.at[2 * c + m])
                    for m, dst in enumerate((wk_v, wv_v))]

        cp_wo = pltpu.make_async_copy(wo_hbm, wo_v, wsem.at[0])
        cp_wq = pltpu.make_async_copy(wqkv_hbm.at[:, pl.ds(0, D)], wq_v, wsem.at[1])

        def cp_ffn(c):
            return (
                pltpu.make_async_copy(w1_hbm.at[:, pl.ds(c * TF, TF)], w1_v.at[c], fsem.at[3 * c]),
                pltpu.make_async_copy(w3_hbm.at[:, pl.ds(c * TF, TF)], w3_v.at[c], fsem.at[3 * c + 1]),
                pltpu.make_async_copy(w2_hbm.at[pl.ds(c * TF, TF), :], w2_v.at[c], fsem.at[3 * c + 2]),
            )

        def gate(x, row0):
            gl = jnp.sum(x.astype(f32) * gw_ref[...].astype(f32), axis=1, keepdims=True)
            g_v[pl.ds(row0, TM), :] = jax.nn.sigmoid(gl)

        def q_cols(x, tix):
            q = jnp.dot(x, wq_v[...], preferred_element_type=f32)
            pqT = _phi(q).T.astype(bf16)
            for c in range(NF):
                pq_v[tix * NF + c] = pqT[c * TA:(c + 1) * TA, :]

        def kv_cols(x, c0, w, first):
            k = jnp.dot(x, wk_v[:, c0:c0 + w], preferred_element_type=f32)
            pkT = _phi(k).T
            zs = pkT[:, 0:_LANE]
            for c in range(1, TM // _LANE):
                zs = zs + pkT[:, c * _LANE:(c + 1) * _LANE]
            if first:
                z_acc[c0:c0 + w, :] = zs
            else:
                z_acc[c0:c0 + w, :] += zs
            pkT = pkT.astype(bf16)
            v = jnp.dot(x, wv_v[:, c0:c0 + w], preferred_element_type=f32).astype(bf16)
            for j in range(w // _LANE):
                sl = slice(j * _LANE, (j + 1) * _LANE)
                gsl = slice(c0 + j * _LANE, c0 + (j + 1) * _LANE)
                t = jnp.dot(pkT[sl, :], v[:, sl], preferred_element_type=f32)
                if first:
                    kv_acc[gsl, :] = t
                else:
                    kv_acc[gsl, :] += t

        @pl.when(jnp.logical_and(p == 0, i == 0))
        def _():
            cp_x(0).start()
            for c in range(min(ahead, NC)):
                for cp in cp_chunk(c):
                    cp.start()
            cp_x(0).wait()
            x = x_v[pl.ds(0, TM), :]
            gate(x, 0)
            for c in range(NC):
                for cp in cp_chunk(c):
                    cp.wait()
                if c + ahead < NC:
                    for cp in cp_chunk(c + ahead):
                        cp.start()
                if c == NC - 2:
                    cp_wq.start()
                if c == NC - 1:
                    cp_x(1).start()
                kv_cols(x, starts[c], widths[c], True)
            cp_wq.wait()
            for t in range(2, NT):
                cp_x(t).start()
            q_cols(x, 0)

        @pl.when(jnp.logical_and(p == 0, i > 0))
        def _():
            cp_x(i).wait()

            @pl.when(i == 1)
            def _():
                cp_wo.start()
                for c in range(NF):
                    for cp in cp_ffn(c):
                        cp.start()

            row0 = pl.multiple_of(i * TM, TM)
            x = x_v[pl.ds(row0, TM), :]
            gate(x, row0)
            q_cols(x, i)
            kv_cols(x, 0, D, False)

        @pl.when(jnp.logical_and(p == 1, i == 0))
        def _():
            cp_wo.wait()
            r = lax.broadcasted_iota(jnp.int32, (_LANE, _LANE), 0) // DH
            c = lax.broadcasted_iota(jnp.int32, (_LANE, _LANE), 1) // DH
            same_head = r == c
            for j in range(NB):
                sl = slice(j * _LANE, (j + 1) * _LANE)
                cc, off = divmod(j * _LANE, TA)
                lsl = slice(off, off + _LANE)
                kvb = jnp.where(same_head, kv_acc[sl, :], 0.0).astype(bf16)
                m_v[cc, lsl, :] = jnp.dot(kvb, wo_v[sl, :], preferred_element_type=f32).astype(bf16)
                z = jnp.sum(z_acc[sl, :], axis=1, keepdims=True)
                zb_v[cc, lsl, :] = jnp.broadcast_to(z.astype(bf16).astype(f32), (_LANE, _LANE))
            for c in range(NF):
                for cp in cp_ffn(c):
                    cp.wait()

        @pl.when(p == 1)
        def _():
            row0 = pl.multiple_of(i * TM, TM)

            def body(c, carry):
                x = x_v[pl.ds(row0, TM), :]
                g = g_v[pl.ds(row0, TM), :]
                pqT = pq_v[i * NF + c].astype(f32)
                zb = zb_v[c]
                zz = jnp.concatenate([zb] * (TM // _LANE), axis=1)
                prod = (pqT * zz).reshape(TA // DH, DH, TM)
                den = jnp.sum(prod, axis=1, keepdims=True) + 1e-6
                pnT = (pqT.reshape(TA // DH, DH, TM) / den).reshape(TA, TM)
                pn = (pnT.T * g).astype(bf16)
                gt = jnp.dot(x, w1_v[c], preferred_element_type=f32)
                up = jnp.dot(x, w3_v[c], preferred_element_type=f32)
                h = (gt * jax.nn.sigmoid(gt) * up * (1.0 - g)).astype(bf16)
                tot = (jnp.where(c > 0, acc[...], 0.0)
                       + jnp.dot(pn, m_v[c], preferred_element_type=f32)
                       + jnp.dot(h, w2_v[c], preferred_element_type=f32))
                acc[...] = tot
                o_ref[...] = tot.astype(o_ref.dtype)
                return carry

            lax.fori_loop(0, NF, body, 0)

    return kernel, NT, NC, TF, TA


@jax.jit
def pallas_gated_mix__linear_attn_block__glu_gated_swiglu__prompt_kernel(
    A_x: jax.Array,
    A_wqkv: jax.Array,
    A_wo: jax.Array,
    B_x: jax.Array,
    B_w1: jax.Array,
    B_w3: jax.Array,
    B_w2: jax.Array,
    gate_w: jax.Array,
):
    B, S, D = A_x.shape
    assert B == 1
    F = B_w1.shape[1]
    TM, NF = 256, 2
    widths = [128, 384, 512]
    kernel, NT, NC, TF, TA = _make_kernel(S, D, F, TM, NF, widths, 2)
    bf16, f32 = jnp.bfloat16, jnp.float32

    x2 = A_x.reshape(S, D)
    gw = gate_w.reshape(1, D)
    any_spec = pl.BlockSpec(memory_space=pl.ANY)
    out = pl.pallas_call(
        kernel,
        grid=(2, NT),
        in_specs=[
            pl.BlockSpec((1, D), lambda p, i: (0, 0)),
            any_spec, any_spec, any_spec, any_spec, any_spec, any_spec,
        ],
        out_specs=pl.BlockSpec((TM, D), lambda p, i: (i * p, 0)),
        out_shape=jax.ShapeDtypeStruct((S, D), A_x.dtype),
        scratch_shapes=[
            pltpu.VMEM((S, D), bf16),
            pltpu.VMEM((NT * NF, TA, TM), bf16),
            pltpu.VMEM((S, 1), f32),
            pltpu.VMEM((D, D), bf16),
            pltpu.VMEM((D, D), bf16),
            pltpu.VMEM((D, D), bf16),
            pltpu.VMEM((D, D), bf16),
            pltpu.VMEM((NF, D, TF), bf16),
            pltpu.VMEM((NF, D, TF), bf16),
            pltpu.VMEM((NF, TF, D), bf16),
            pltpu.VMEM((D, _LANE), f32),
            pltpu.VMEM((D, _LANE), f32),
            pltpu.VMEM((NF, TA, D), bf16),
            pltpu.VMEM((NF, TA, _LANE), f32),
            pltpu.VMEM((TM, D), f32),
            pltpu.SemaphoreType.DMA((NT,)),
            pltpu.SemaphoreType.DMA((2 * NC,)),
            pltpu.SemaphoreType.DMA((2,)),
            pltpu.SemaphoreType.DMA((3 * NF,)),
        ],
        compiler_params=pltpu.CompilerParams(
            dimension_semantics=("arbitrary", "arbitrary"),
            vmem_limit_bytes=100 * 1024 * 1024,
        ),
    )(gw, x2, A_wqkv, A_wo, B_w1, B_w3, B_w2)
    return out.reshape(B, S, D)
```
